```python
import os as _os
_os.environ.setdefault("JAX_PLATFORMS", "cpu")
import jax
import jax.numpy as jnp

def _softmax(x, axis=-1):
    return jax.nn.softmax(x, axis=axis)
def _gelu(x):
    return jax.nn.gelu(x, approximate=True)
def _silu(x):
    return jax.nn.silu(x)
def _sigmoid(x):
    return jax.nn.sigmoid(x)
def _layernorm(x, axis=-1, eps=1e-5):
    m = jnp.mean(x, axis=axis, keepdims=True)
    v = jnp.var(x, axis=axis, keepdims=True)
    return (x - m) / jnp.sqrt(v + eps)
def _scatter_add(tgt, idx, src, axis=0):
    return tgt.at[idx].add(src)
def _segment_sum(src, seg, n):
    return jax.ops.segment_sum(src, seg, n)
class _Rng:
    def __init__(self, key):
        self._k = key
    def _next(self):
        self._k, sub = jax.random.split(self._k)
        return sub
    def normal(self, shape):
        return jax.random.normal(self._next(), shape, dtype=jnp.bfloat16)
    def randint(self, lo, hi, shape):
        return jax.random.randint(self._next(), shape, lo, hi, dtype=jnp.int32)
    def uniform(self, shape, lo=0.0, hi=1.0):
        return jax.random.uniform(self._next(), shape, jnp.bfloat16, lo, hi)
    def permutation(self, n):
        return jax.random.permutation(self._next(), n)


kernel_name = 'sequential_preLN__sliding_local_dilated__dense_activation_relu__prompt'

def setup_inputs():
    _rng = _Rng(jax.random.key(int.from_bytes(__import__("os").urandom(4), "little")))
    _w = (lambda a: (lambda t: t.astype(jnp.bfloat16) if jnp.issubdtype(t.dtype, jnp.floating) else t)(jnp.asarray(a)))
    def _A_setup():
        B, S, D = 1, 2048, 1024
        return {
            "x": _w((lambda *s: _rng.normal(s) * 0.05)(B, S, D)),
            "wqkv": _w((lambda *s: _rng.normal(s) * 0.05)(D, 3 * D)),
            "wo": _w((lambda *s: _rng.normal(s) * 0.05)(D, D)),
        }
    _A_in = _A_setup()

    def _B_setup():
        B, S, D, Dff = 1, 2048, 1024, 3584
        return {
            "x": _w((lambda *s: _rng.normal(s) * 0.05)(B, S, D)),
            "w1": _w((lambda *s: _rng.normal(s) * 0.05)(D, Dff)),
            "w2": _w((lambda *s: _rng.normal(s) * 0.05)(Dff, D)),
        }
    _B_in = _B_setup()

    return {
        "A_x": _A_in["x"],
        "A_wqkv": _A_in["wqkv"],
        "A_wo": _A_in["wo"],
        "B_x": _B_in["x"],
        "B_w1": _B_in["w1"],
        "B_w2": _B_in["w2"],
    }

def reference(A_x, A_wqkv, A_wo, B_x, B_w1, B_w2):
    def _A_ref(x, wqkv, wo):
        B, S, D = x.shape
        H = 32; Dh = D // H
        W, dil = 8, 2
        qkv = (lambda x, *d: x.transpose(*d))((x @ wqkv).reshape(B, S, 3, H, Dh), 2, 0, 3, 1, 4)
        q, k, v = qkv[0], qkv[1], qkv[2]
        scale = Dh ** -0.5
        pos = jnp.arange(S)
        off = jnp.arange(W) * dil
        idx = pos[:, None] - off[None, :]
        mask = idx >= 0
        idx_c = jnp.where(mask, idx, 0).reshape(-1)
        kg = k[:, :, idx_c, :].reshape(B, H, S, W, Dh)
        vg = v[:, :, idx_c, :].reshape(B, H, S, W, Dh)
        logits = jnp.einsum("bhsd,bhswd->bhsw", q, kg) * scale
        logits = jnp.where(mask[None, None, :, :], logits, -1e9)
        attn = _softmax(logits, axis=-1)
        o = jnp.einsum("bhsw,bhswd->bhsd", attn, vg)
        return (lambda x, *d: x.transpose(*d))(o, 0, 2, 1, 3).reshape(B, S, D) @ wo

    def _B_ref(x, w1, w2):
        h = jnp.einsum("bsd,df->bsf", x, w1)
        zero = jnp.zeros_like(h)
        h = jnp.maximum(h, zero)
        return jnp.einsum("bsf,fd->bsd", h, w2)

    x = A_x
    h = x + _A_ref(_layernorm(x, axis=-1), A_wqkv, A_wo)
    h2 = h + _B_ref(_layernorm(h, axis=-1), B_w1, B_w2)
    return h2
```

```python
import functools
import jax
import jax.numpy as jnp
from jax import lax
import jax.experimental.pallas as pl
import jax.experimental.pallas.tpu as pltpu

H = 32
WIN = 8
DIL = 2
HALO = 16
EPS = 1e-5
NEG = -1e9
TM = 256
RB = 8
LRB = 16
RBP = 32
FCH = 512
TOK = 7


def _ln(x):
    m = jnp.mean(x, axis=-1, keepdims=True)
    xc = x - m
    v = jnp.mean(xc * xc, axis=-1, keepdims=True)
    return xc * lax.rsqrt(v + EPS)


def _nt_dot(a, b):
    return lax.dot_general(a, b, (((1,), (1,)), ((), ())), preferred_element_type=jnp.float32)


def _kernel(xnext_ref, xcur_ref, wqkv_hbm, wo_hbm, w1_hbm, w2_hbm, o_ref,
            wqkv_v, wt_v, wo_raw, wo_v, w1_v, w2_v, kbuf, vbuf, qbuf, xn_buf, o_buf, h_buf, hn_buf, acc_buf,
            flag_ref, sems, *, tm, d, dff, nt):
    i = pl.program_id(0)
    dh = d // H
    scale = dh ** -0.5
    f32 = jnp.float32
    bf16 = jnp.bfloat16
    g = dh // 8

    nkb = d // 128

    def qkv_copy(kb):
        return pltpu.make_async_copy(wqkv_hbm.at[pl.ds(kb * 128, 128), :], wqkv_v.at[pl.ds(kb * 128, 128), :], sems.at[3 + kb])

    wo_copy = pltpu.make_async_copy(wo_hbm, wo_raw, sems.at[0])
    w1_copy = pltpu.make_async_copy(w1_hbm, w1_v, sems.at[1])
    w2_copy = pltpu.make_async_copy(w2_hbm, w2_v, sems.at[2])
    copies = [qkv_copy(kb) for kb in range(nkb)] + [wo_copy, w1_copy, w2_copy]

    def chain(tok, x):
        if tok is None:
            return x
        reps = x.shape[1] // tok.shape[1]
        if reps > 1:
            tok = jnp.concatenate([tok] * reps, axis=1)
        return jnp.where(flag_ref[0] != 0, tok, x)

    def permute_rows(t):
        n = t.shape[1]
        return t.reshape(H // 8, 8, g, 8, n).transpose(2, 3, 0, 1, 4).reshape(d, n)

    def prep_wqkv(kb, carry):
        r0 = pl.multiple_of(kb * 128, 128)
        qkv_copy(kb).wait()
        for sec in range(3):
            wt = jnp.transpose(wqkv_v[pl.ds(r0, 128), sec * d:(sec + 1) * d].astype(f32))
            wt_v[sec * d:(sec + 1) * d, pl.ds(r0, 128)] = permute_rows(wt).astype(bf16)
        return carry

    def prep_wo():
        for nb in range(d // 128):
            t = wo_raw[:, nb * 128:(nb + 1) * 128].astype(f32)
            wo_v[:, nb * 128:(nb + 1) * 128] = permute_rows(t).astype(bf16)

    def attention_rows(r0, first, tok, RB=RB):
        dyn = not isinstance(r0, int)
        q = qbuf[pl.ds(r0, RB), :]
        if dyn:
            kwin = kbuf[pl.ds(r0, RB + HALO), :]
            vwin = vbuf[pl.ds(r0, RB + HALO), :]
        logits = []
        for w in range(WIN):
            off = w * DIL
            kw = kwin[HALO - off:HALO - off + RB] if dyn else kbuf[pl.ds(HALO - off + r0, RB), :]
            p = chain(tok, q) * kw
            s = p[:, 0:128]
            for j in range(1, d // 128):
                s = s + p[:, j * 128:(j + 1) * 128]
            tok = s if (TOK & 1) and not dyn else None
            s = s + pltpu.roll(s, 32, 1)
            s = s + pltpu.roll(s, 64, 1)
            if first and w > 0:
                row = r0 + lax.broadcasted_iota(jnp.int32, (RB, 128), 0)
                s = jnp.where(row >= off, s, NEG)
            logits.append(s)
        m = logits[0]
        for w in range(1, WIN):
            m = jnp.maximum(m, logits[w])
        es = [jnp.exp(l - m) for l in logits]
        den = es[0]
        for w in range(1, WIN):
            den = den + es[w]
        inv = 1.0 / den
        acc = None
        for w in range(WIN):
            off = w * DIL
            e8 = jnp.concatenate([es[w] * inv] * (d // 128), axis=1)
            vw = vwin[HALO - off:HALO - off + RB] if dyn else vbuf[pl.ds(HALO - off + r0, RB), :]
            t = e8 * vw
            acc = t if acc is None else acc + t
        o_buf[pl.ds(r0, RB), :] = acc.astype(bf16)
        return acc if (TOK & 2) and not dyn else None

    def carry_halo():
        kbuf[0:HALO, :] = kbuf[tm:tm + HALO, :]
        vbuf[0:HALO, :] = vbuf[tm:tm + HALO, :]

    def out_proj():
        return xcur_ref[...].astype(f32) + jnp.dot(o_buf[...], wo_v[...], preferred_element_type=f32)

    def ln_rows(src, dst_ref, tok):
        for r0 in range(0, tm, LRB):
            y = _ln(chain(tok, src(r0)))
            dst_ref[r0:r0 + LRB, :] = y.astype(bf16)
            tok = y if (TOK & 4) else None
        return tok

    @pl.when(i == 0)
    def _():
        for c in copies:
            c.start()
        flag_ref[0] = 0
        kbuf[0:HALO, :] = jnp.zeros((HALO, d), f32)
        vbuf[0:HALO, :] = jnp.zeros((HALO, d), f32)
        xn_buf[...] = _ln(xcur_ref[...].astype(f32)).astype(bf16)
        lax.fori_loop(0, nkb, prep_wqkv, 0)

    @pl.when(i < nt)
    def _():
        xn = xn_buf[...]
        qbuf[...] = _nt_dot(xn, wt_v[0:d, :]) * scale
        kbuf[HALO:HALO + tm, :] = _nt_dot(xn, wt_v[d:2 * d, :])
        vbuf[HALO:HALO + tm, :] = _nt_dot(xn, wt_v[2 * d:3 * d, :])

    @pl.when(i == 0)
    def _():
        def b1(j, c):
            attention_rows(pl.multiple_of(j * RBP, RBP), True, None, RBP)
            return c
        lax.fori_loop(0, tm // RBP, b1, 0)
        carry_halo()
        wo_copy.wait()
        prep_wo()
        h = out_proj()
        h_buf[...] = h
        hn_buf[...] = _ln(h).astype(bf16)
        xn_buf[...] = _ln(xnext_ref[...].astype(f32)).astype(bf16)

    @pl.when(i == 1)
    def _():
        w1_copy.wait()
        w2_copy.wait()

    @pl.when(jnp.logical_and(i > 0, i < nt))
    def _():
        hprev = h_buf[...]
        a = jnp.maximum(jnp.dot(hn_buf[...], w1_v[...], preferred_element_type=f32), 0.0).astype(bf16)
        tok = None
        for r0 in range(0, tm, RB):
            tok = attention_rows(r0, False, tok)
        carry_halo()
        h = out_proj()
        h_buf[...] = h
        y = hprev + jnp.dot(a, w2_v[...], preferred_element_type=f32)
        o_ref[...] = y.astype(o_ref.dtype)
        tok = ln_rows(lambda r0: h[r0:r0 + LRB], hn_buf, None)
        ln_rows(lambda r0: xnext_ref[r0:r0 + LRB, :].astype(f32), xn_buf, tok)

    @pl.when(i == nt)
    def _():
        acc_buf[...] = h_buf[...]

        def body(j, carry):
            c0 = pl.multiple_of(j * FCH, FCH)
            a = jnp.maximum(jnp.dot(hn_buf[...], w1_v[:, pl.ds(c0, FCH)], preferred_element_type=f32), 0.0).astype(bf16)
            acc_buf[...] += jnp.dot(a, w2_v[pl.ds(c0, FCH), :], preferred_element_type=f32)
            return carry

        lax.fori_loop(0, dff // FCH, body, 0)
        o_ref[...] = acc_buf[...].astype(o_ref.dtype)


@jax.jit
def pallas_sequential_preLN__sliding_local_dilated__dense_activation_relu__prompt_kernel(
    A_x, A_wqkv, A_wo, B_x, B_w1, B_w2,
):
    b, s, d = A_x.shape
    dff = B_w1.shape[1]
    assert b == 1
    tm = TM
    nt = s // tm
    x2 = A_x.reshape(s, d)
    kern = functools.partial(_kernel, tm=tm, d=d, dff=dff, nt=nt)
    out = pl.pallas_call(
        kern,
        grid=(nt + 1,),
        in_specs=[
            pl.BlockSpec((tm, d), lambda i: (jnp.minimum(i + 1, nt - 1), 0)),
            pl.BlockSpec((tm, d), lambda i: (jnp.minimum(i, nt - 1), 0)),
            pl.BlockSpec(memory_space=pl.ANY),
            pl.BlockSpec(memory_space=pl.ANY),
            pl.BlockSpec(memory_space=pl.ANY),
            pl.BlockSpec(memory_space=pl.ANY),
        ],
        out_specs=pl.BlockSpec((tm, d), lambda i: (jnp.maximum(i - 1, 0), 0)),
        out_shape=jax.ShapeDtypeStruct((s, d), A_x.dtype),
        scratch_shapes=[
            pltpu.VMEM((d, 3 * d), jnp.bfloat16),
            pltpu.VMEM((3 * d, d), jnp.bfloat16),
            pltpu.VMEM((d, d), jnp.bfloat16),
            pltpu.VMEM((d, d), jnp.bfloat16),
            pltpu.VMEM((d, dff), jnp.bfloat16),
            pltpu.VMEM((dff, d), jnp.bfloat16),
            pltpu.VMEM((tm + HALO, d), jnp.float32),
            pltpu.VMEM((tm + HALO, d), jnp.float32),
            pltpu.VMEM((tm, d), jnp.float32),
            pltpu.VMEM((tm, d), jnp.bfloat16),
            pltpu.VMEM((tm, d), jnp.bfloat16),
            pltpu.VMEM((tm, d), jnp.float32),
            pltpu.VMEM((tm, d), jnp.bfloat16),
            pltpu.VMEM((tm, d), jnp.float32),
            pltpu.SMEM((1,), jnp.int32),
            pltpu.SemaphoreType.DMA((3 + d // 128,)),
        ],
        compiler_params=pltpu.CompilerParams(
            dimension_semantics=("arbitrary",),
            vmem_limit_bytes=100 * 1024 * 1024,
        ),
    )(x2, x2, A_wqkv, A_wo, B_w1, B_w2)
    return out.reshape(b, s, d)
```

```python
import functools

import jax
import jax.numpy as jnp
from jax import lax
import jax.experimental.pallas as pl
import jax.experimental.pallas.tpu as pltpu

H = 32
WIN = 8
DIL = 2
HALO = 16
EPS = 1e-5
NEG = -1e9
TM = 256
RB = 8
RBP = 32
LRB = 16
FCH = 512


def _ln(x):
    m = jnp.mean(x, axis=-1, keepdims=True)
    xc = x - m
    v = jnp.mean(xc * xc, axis=-1, keepdims=True)
    return xc * lax.rsqrt(v + EPS)


def _nt_dot(a, b):
    return lax.dot_general(a, b, (((1,), (1,)), ((), ())), preferred_element_type=jnp.float32)


def _kernel(xnext_ref, xcur_ref, wqkv_hbm, wo_hbm, w1_hbm, w2_hbm, o_ref,
            wqkv_v, wt_v, wo_raw, wo_v, w1_v, w2_v, kbuf, vbuf, qbuf, xn_buf, o_buf, h_buf, hn_buf,
            acc_buf, st_a, st_b, flag_ref, sems, *, tm, d, dff, nt):
    i = pl.program_id(0)
    dh = d // H
    scale = dh ** -0.5
    f32 = jnp.float32
    bf16 = jnp.bfloat16
    nkb = d // 128

    def qkv_copy(kb):
        return pltpu.make_async_copy(wqkv_hbm.at[pl.ds(kb * 128, 128), :],
                                     wqkv_v.at[pl.ds(kb * 128, 128), :], sems.at[3 + kb])

    wo_copy = pltpu.make_async_copy(wo_hbm, wo_raw, sems.at[0])
    w1_copy = pltpu.make_async_copy(w1_hbm, w1_v, sems.at[1])
    w2_copy = pltpu.make_async_copy(w2_hbm, w2_v, sems.at[2])

    def chain(tok, x):
        if tok is None:
            return x
        reps = x.shape[1] // tok.shape[1]
        if reps > 1:
            tok = jnp.concatenate([tok] * reps, axis=1)
        return jnp.where(flag_ref[0] != 0, tok, x)

    def permute_rows(t):
        n = t.shape[1]
        return t.reshape(H // 8, 8, dh // 8, 8, n).transpose(2, 3, 0, 1, 4).reshape(d, n)

    def prep_wqkv(kb, st):
        r0 = kb * 128 if isinstance(kb, int) else pl.multiple_of(kb * 128, 128)
        qkv_copy(kb).wait()
        tok = None
        for sec in range(3):
            wt = jnp.transpose(chain(tok, wqkv_v[pl.ds(r0, 128), sec * d:(sec + 1) * d].astype(f32)))
            wp32 = permute_rows(wt)
            wp = wp32.astype(bf16)
            wt_v[sec * d:(sec + 1) * d, pl.ds(r0, 128)] = wp
            st[sec * d:(sec + 1) * d, :] = wp
            tok = wp32[d - 128:d, :]

    def partial_qkv(kb, st):
        r0 = kb * 128 if isinstance(kb, int) else pl.multiple_of(kb * 128, 128)
        xk = xn_buf[:, pl.ds(r0, 128)]
        qbuf[...] += _nt_dot(xk, st[0:d, :])
        kbuf[0, HALO:HALO + tm, :] += _nt_dot(xk, st[d:2 * d, :])
        vbuf[0, HALO:HALO + tm, :] += _nt_dot(xk, st[2 * d:3 * d, :])

    def prep_and_dot(p, carry):
        prep_wqkv(2 * p + 1, st_b)
        partial_qkv(2 * p, st_a)
        prep_wqkv(2 * p + 2, st_a)
        partial_qkv(2 * p + 1, st_b)
        return carry

    def prep_wo():
        for nb in range(d // 128):
            t = wo_raw[:, nb * 128:(nb + 1) * 128].astype(f32)
            wo_v[:, nb * 128:(nb + 1) * 128] = permute_rows(t).astype(bf16)

    def put(buf, val, b0):
        for bi in range(b0, 4):
            buf[bi, HALO + 2 * bi:HALO + 2 * bi + tm, :] = val

    def window(buf, r0, w, rb):
        off = w * DIL
        return buf[(off % 8) // 2, pl.ds(HALO + r0 - 8 * (off // 8), rb), :]

    def attention_rows(r0, rb, first, tok):
        q = qbuf[pl.ds(r0, rb), :]
        logits = []
        for w in range(WIN):
            p = (chain(tok, q) if w == 0 else q) * window(kbuf, r0, w, rb)
            s = p[:, 0:128]
            for j in range(1, d // 128):
                s = s + p[:, j * 128:(j + 1) * 128]
            s = s + pltpu.roll(s, 32, 1)
            s = s + pltpu.roll(s, 64, 1)
            if first and w > 0:
                row = r0 + lax.broadcasted_iota(jnp.int32, (rb, 128), 0)
                s = jnp.where(row >= w * DIL, s, NEG)
            logits.append(s)
        m = logits[0]
        for w in range(1, WIN):
            m = jnp.maximum(m, logits[w])
        es = [jnp.exp(l - m) for l in logits]
        den = es[0]
        for w in range(1, WIN):
            den = den + es[w]
        inv = 1.0 / den
        acc = None
        for w in range(WIN):
            e8 = jnp.concatenate([es[w] * inv] * (d // 128), axis=1)
            if not first:
                e8 = chain(acc, e8)
            t = e8 * window(vbuf, r0, w, rb)
            acc = t if acc is None else acc + t
        o_buf[pl.ds(r0, rb), :] = acc.astype(bf16)
        return acc

    def carry_halo():
        kbuf[:, 0:HALO + 8, :] = kbuf[:, tm:tm + HALO + 8, :]
        vbuf[:, 0:HALO + 8, :] = vbuf[:, tm:tm + HALO + 8, :]

    def out_proj():
        return xcur_ref[...].astype(f32) + jnp.dot(o_buf[...], wo_v[...], preferred_element_type=f32)

    def ln_rows(src, dst_ref, tok):
        for r0 in range(0, tm, LRB):
            tok = _ln(chain(tok, src(r0)))
            dst_ref[r0:r0 + LRB, :] = tok.astype(bf16)
        return tok

    @pl.when(i == 0)
    def _():
        for kb in range(nkb):
            qkv_copy(kb).start()
        wo_copy.start()
        w1_copy.start()
        w2_copy.start()
        flag_ref[0] = 0
        for buf in (kbuf, vbuf):
            buf[0] = jnp.zeros(buf.shape[1:], f32)
            buf[1:4, 0:HALO + 8, :] = jnp.zeros((3, HALO + 8, d), f32)
            buf[1:4, tm + HALO:tm + HALO + 8, :] = jnp.zeros((3, 8, d), f32)
        qbuf[...] = jnp.zeros((tm, d), f32)
        xn_buf[...] = _ln(xcur_ref[...].astype(f32)).astype(bf16)
        prep_wqkv(0, st_a)
        lax.fori_loop(0, nkb // 2 - 1, prep_and_dot, 0)
        prep_wqkv(nkb - 1, st_b)
        partial_qkv(nkb - 2, st_a)
        partial_qkv(nkb - 1, st_b)
        qbuf[...] = qbuf[...] * scale
        put(kbuf, kbuf[0, HALO:HALO + tm, :], 1)
        put(vbuf, vbuf[0, HALO:HALO + tm, :], 1)

    @pl.when(jnp.logical_and(i > 0, i < nt))
    def _():
        xn = xn_buf[...]
        qbuf[...] = _nt_dot(xn, wt_v[0:d, :]) * scale
        put(kbuf, _nt_dot(xn, wt_v[d:2 * d, :]), 0)
        put(vbuf, _nt_dot(xn, wt_v[2 * d:3 * d, :]), 0)

    @pl.when(i == 0)
    def _():
        def body(j, c):
            attention_rows(pl.multiple_of(j * RBP, RBP), RBP, True, None)
            return c
        lax.fori_loop(0, tm // RBP, body, 0)
        carry_halo()
        wo_copy.wait()
        prep_wo()
        h = out_proj()
        h_buf[...] = h
        hn_buf[...] = _ln(h).astype(bf16)
        xn_buf[...] = _ln(xnext_ref[...].astype(f32)).astype(bf16)

    @pl.when(i == 1)
    def _():
        w1_copy.wait()
        w2_copy.wait()

    @pl.when(jnp.logical_and(i > 0, i < nt))
    def _():
        hprev = h_buf[...]
        a = jnp.maximum(jnp.dot(hn_buf[...], w1_v[...], preferred_element_type=f32), 0.0).astype(bf16)
        tok = None
        for r0 in range(0, tm, RB):
            tok = attention_rows(r0, RB, False, tok)
        carry_halo()
        h = out_proj()
        h_buf[...] = h
        y = hprev + jnp.dot(a, w2_v[...], preferred_element_type=f32)
        o_ref[...] = y.astype(o_ref.dtype)
        tok = ln_rows(lambda r0: h[r0:r0 + LRB], hn_buf, None)
        ln_rows(lambda r0: xnext_ref[r0:r0 + LRB, :].astype(f32), xn_buf, tok)

    @pl.when(i == nt)
    def _():
        acc_buf[...] = h_buf[...]

        def body(j, carry):
            c0 = pl.multiple_of(j * FCH, FCH)
            a = jnp.maximum(jnp.dot(hn_buf[...], w1_v[:, pl.ds(c0, FCH)], preferred_element_type=f32),
                            0.0).astype(bf16)
            acc_buf[...] += jnp.dot(a, w2_v[pl.ds(c0, FCH), :], preferred_element_type=f32)
            return carry

        lax.fori_loop(0, dff // FCH, body, 0)
        o_ref[...] = acc_buf[...].astype(o_ref.dtype)


@jax.jit
def pallas_sequential_preLN__sliding_local_dilated__dense_activation_relu__prompt_kernel(
    A_x: jax.Array,
    A_wqkv: jax.Array,
    A_wo: jax.Array,
    B_x: jax.Array,
    B_w1: jax.Array,
    B_w2: jax.Array,
):
    b, s, d = A_x.shape
    dff = B_w1.shape[1]
    tm = TM
    nt = s // tm
    assert b == 1 and s % tm == 0 and nt >= 2 and d == 32 * H and dff % FCH == 0
    x2 = A_x.reshape(s, d)
    bf16, f32 = jnp.bfloat16, jnp.float32
    kern = functools.partial(_kernel, tm=tm, d=d, dff=dff, nt=nt)
    out = pl.pallas_call(
        kern,
        grid=(nt + 1,),
        in_specs=[
            pl.BlockSpec((tm, d), lambda i: (jnp.minimum(i + 1, nt - 1), 0)),
            pl.BlockSpec((tm, d), lambda i: (jnp.minimum(i, nt - 1), 0)),
            pl.BlockSpec(memory_space=pl.ANY),
            pl.BlockSpec(memory_space=pl.ANY),
            pl.BlockSpec(memory_space=pl.ANY),
            pl.BlockSpec(memory_space=pl.ANY),
        ],
        out_specs=pl.BlockSpec((tm, d), lambda i: (jnp.maximum(i - 1, 0), 0)),
        out_shape=jax.ShapeDtypeStruct((s, d), A_x.dtype),
        scratch_shapes=[
            pltpu.VMEM((d, 3 * d), bf16),
            pltpu.VMEM((3 * d, d), bf16),
            pltpu.VMEM((d, d), bf16),
            pltpu.VMEM((d, d), bf16),
            pltpu.VMEM((d, dff), bf16),
            pltpu.VMEM((dff, d), bf16),
            pltpu.VMEM((4, tm + HALO + 8, d), f32),
            pltpu.VMEM((4, tm + HALO + 8, d), f32),
            pltpu.VMEM((tm, d), f32),
            pltpu.VMEM((tm, d), bf16),
            pltpu.VMEM((tm, d), bf16),
            pltpu.VMEM((tm, d), f32),
            pltpu.VMEM((tm, d), bf16),
            pltpu.VMEM((tm, d), f32),
            pltpu.VMEM((3 * d, 128), bf16),
            pltpu.VMEM((3 * d, 128), bf16),
            pltpu.SMEM((1,), jnp.int32),
            pltpu.SemaphoreType.DMA((3 + d // 128,)),
        ],
        compiler_params=pltpu.CompilerParams(
            dimension_semantics=("arbitrary",),
            vmem_limit_bytes=100 * 1024 * 1024,
        ),
    )(x2, x2, A_wqkv, A_wo, B_w1, B_w2)
    return out.reshape(b, s, d)
```
